```python
import os as _os
_os.environ.setdefault("JAX_PLATFORMS", "cpu")
import jax
import jax.numpy as jnp

def _softmax(x, axis=-1):
    return jax.nn.softmax(x, axis=axis)
def _gelu(x):
    return jax.nn.gelu(x, approximate=True)
def _silu(x):
    return jax.nn.silu(x)
def _sigmoid(x):
    return jax.nn.sigmoid(x)
def _layernorm(x, axis=-1, eps=1e-5):
    m = jnp.mean(x, axis=axis, keepdims=True)
    v = jnp.var(x, axis=axis, keepdims=True)
    return (x - m) / jnp.sqrt(v + eps)
def _scatter_add(tgt, idx, src, axis=0):
    return tgt.at[idx].add(src)
def _segment_sum(src, seg, n):
    return jax.ops.segment_sum(src, seg, n)
class _Rng:
    def __init__(self, key):
        self._k = key
    def _next(self):
        self._k, sub = jax.random.split(self._k)
        return sub
    def normal(self, shape):
        return jax.random.normal(self._next(), shape, dtype=jnp.bfloat16)
    def randint(self, lo, hi, shape):
        return jax.random.randint(self._next(), shape, lo, hi, dtype=jnp.int32)
    def uniform(self, shape, lo=0.0, hi=1.0):
        return jax.random.uniform(self._next(), shape, jnp.bfloat16, lo, hi)
    def permutation(self, n):
        return jax.random.permutation(self._next(), n)


kernel_name = 'sequential_preLN__linear_attn_block__glu_gated_reglu__prompt'

def setup_inputs():
    _rng = _Rng(jax.random.key(int.from_bytes(__import__("os").urandom(4), "little")))
    _w = (lambda a: (lambda t: t.astype(jnp.bfloat16) if jnp.issubdtype(t.dtype, jnp.floating) else t)(jnp.asarray(a)))
    def _A_setup():
        B, S, D = 1, 2048, 640
        return {
            "x": _w((lambda *s: _rng.normal(s) * 0.05)(B, S, D)),
            "wqkv": _w((lambda *s: _rng.normal(s) * 0.05)(D, 3 * D)),
            "wo": _w((lambda *s: _rng.normal(s) * 0.05)(D, D)),
        }
    _A_in = _A_setup()

    def _B_setup():
        B, S, D, F = 1, 2048, 640, 1536
        return {
            "x": _w((lambda *s: _rng.normal(s) * 0.05)(B, S, D)),
            "W_gate": _w((lambda *s: _rng.normal(s) * 0.05)(D, F) * (2.0 / D) ** 0.5),
            "W_up": _w((lambda *s: _rng.normal(s) * 0.05)(D, F) * (2.0 / D) ** 0.5),
            "W_down": _w((lambda *s: _rng.normal(s) * 0.05)(F, D) * (1.0 / F) ** 0.5),
        }
    _B_in = _B_setup()

    return {
        "A_x": _A_in["x"],
        "A_wqkv": _A_in["wqkv"],
        "A_wo": _A_in["wo"],
        "B_x": _B_in["x"],
        "B_W_gate": _B_in["W_gate"],
        "B_W_up": _B_in["W_up"],
        "B_W_down": _B_in["W_down"],
    }

def reference(A_x, A_wqkv, A_wo, B_x, B_W_gate, B_W_up, B_W_down):
    def _A_ref(x, wqkv, wo):
        B, S, D = x.shape
        H = 32; Dh = D // H
        qkv = (lambda x, *d: x.transpose(*d))((x @ wqkv).reshape(B, S, 3, H, Dh), 2, 0, 3, 1, 4)
        q, k, v = qkv[0], qkv[1], qkv[2]
        phi = lambda t: jnp.where(t > 0, t + 1, jnp.exp(t)) + 1e-6
        pq, pk = phi(q), phi(k)
        kv = jnp.einsum("bhsd,bhse->bhde", pk, v)
        z = jnp.einsum("bhsd->bhd", pk)
        num = jnp.einsum("bhqd,bhde->bhqe", pq, kv)
        den = jnp.einsum("bhqd,bhd->bhq", pq, z)[..., None] + 1e-6
        o = num / den
        return (lambda x, *d: x.transpose(*d))(o, 0, 2, 1, 3).reshape(B, S, D) @ wo

    def _B_ref(x, W_gate, W_up, W_down):
        gate = jnp.einsum("bsd,df->bsf", x, W_gate)
        up = jnp.einsum("bsd,df->bsf", x, W_up)
        gate = gate * (lambda x, dt: x.astype(dt))(gate > 0, gate.dtype)
        h = gate * up
        return jnp.einsum("bsf,fd->bsd", h, W_down)

    x = A_x
    h = x + _A_ref(_layernorm(x, axis=-1), A_wqkv, A_wo)
    h2 = h + _B_ref(_layernorm(h, axis=-1), B_W_gate, B_W_up, B_W_down)
    return h2
```

```python
import jax
import jax.numpy as jnp
import jax.experimental.pallas as pl
import jax.experimental.pallas.tpu as pltpu
from jax import lax

S, D, F, DH = 2048, 640, 1536, 20
T = 256
N = S // T
LC = 32
AHEAD = 3
BF = jnp.bfloat16
F32 = jnp.float32
NT = (((1,), (1,)), ((), ()))
TN = (((0,), (0,)), ((), ()))
RNG = [(0, 144), (112, 272), (240, 400), (368, 528), (496, 640)]


def _ln(x):
    m = jnp.mean(x, axis=-1, keepdims=True)
    xc = x - m
    v = jnp.mean(xc * xc, axis=-1, keepdims=True)
    return xc * lax.rsqrt(v + 1e-5)


def _phi(t):
    return jnp.where(t > 0, t + 1.0, jnp.exp(t)) + 1e-6


def _dot(a, b):
    return jnp.dot(a, b, preferred_element_type=F32)


def _recip(d):
    r = pl.reciprocal(d, approx=True)
    return r * (2.0 - d * r)


def _head(i):
    return (i * 3277) >> 16


def _kernel(x_hbm, wqkv_hbm, wo_hbm, wg_hbm, wu_hbm, wd_hbm, out_hbm,
            x_v, wq_v, wk_v, wv_v, wo_v, wg_v, wu_v, wd_v,
            wqT_v, wkT_v, xn_v, m_v, zb_v, h_v, hn_v, o_v, sems, osems):
    cp = pltpu.make_async_copy
    cxa = cp(x_hbm.at[0:T], x_v.at[0:T], sems.at[0])
    cxb = cp(x_hbm.at[T:2 * T], x_v.at[T:2 * T], sems.at[1])
    cxc = cp(x_hbm.at[2 * T:S], x_v.at[2 * T:S], sems.at[2])
    cwq = cp(wqkv_hbm.at[:, 0:D], wq_v, sems.at[3])
    cwk = cp(wqkv_hbm.at[:, D:2 * D], wk_v, sems.at[4])
    cwv = cp(wqkv_hbm.at[:, 2 * D:3 * D], wv_v, sems.at[5])
    cwo = cp(wo_hbm, wo_v, sems.at[6])
    cwg = cp(wg_hbm, wg_v, sems.at[7])
    cwu = cp(wu_hbm, wu_v, sems.at[8])
    cwd = cp(wd_hbm, wd_v, sems.at[9])

    def lnx(t):
        cs = []
        for c in range(T // LC):
            r = pl.ds(t * T + c * LC, LC)
            xc = _ln(x_v[r, :].astype(F32)).astype(BF)
            xn_v[r, :] = xc
            cs.append(xc)
        return jnp.concatenate(cs, axis=0)

    st = {"g": None, "z": None}

    def kproj(xn):
        pk = _phi(lax.dot_general(wkT_v[...], xn, NT, preferred_element_type=F32))
        for c in range(T // 128):
            zt = pk[:, c * 128:(c + 1) * 128]
            st["z"] = zt if st["z"] is None else st["z"] + zt
        return pk.astype(BF)

    def gacc(pk, xn):
        gg = _dot(pk, xn)
        st["g"] = gg if st["g"] is None else st["g"] + gg

    def tie_to(dst, src):
        acc = None
        for i in range(src.shape[0] // 16):
            for j in range(src.shape[1] // 128):
                w = pltpu.bitcast(src[i * 16:(i + 1) * 16, j * 128:(j + 1) * 128], jnp.int32)
                acc = w if acc is None else acc | w
        zero = pl.program_id(0)
        n = dst.shape[0]
        d0 = pltpu.bitcast(pltpu.bitcast(dst[n - 16:n, 0:128], jnp.int32) | (acc & zero), BF)
        bot = jnp.concatenate([d0, dst[n - 16:n, 128:]], axis=1)
        return jnp.concatenate([dst[0:n - 16], bot], axis=0)

    cxa.start()
    cwk.start()
    cxa.wait()
    cxb.start()
    xn_first = lnx(0)
    cwk.wait()
    cxb.wait()
    cxc.start()
    wkT_v[...] = wk_v[...].T

    pend = None
    for t in range(N):
        xn = xn_first if t == 0 else None
        if t == 1:
            for c in (cwq, cwv, cwo):
                c.start()
        if t == 2:
            cxc.wait()
            for c in (cwg, cwu, cwd):
                c.start()
        if t == N - 2:
            xn = lnx(t)
            gacc(tie_to(pend[0], xn), pend[1])
            pend = None
            for c in (cwq, cwv, cwo):
                c.wait()
        if pend is not None:
            gacc(*pend)
        if xn is None:
            xn = lnx(t)
        pk = kproj(xn)
        if t == N - 2:
            wqT_v[...] = wq_v[...].T
        pend = (pk, xn)
    gacc(*pend)

    def qproj(t):
        return _phi(lax.dot_general(wqT_v[...], xn_v[pl.ds(t * T, T), :], NT,
                                    preferred_element_type=F32))

    def attn(t, pq):
        low = lax.broadcasted_iota(jnp.int32, (16, 8, 128), 1) < 4
        cols = []
        for c in range(T // 128):
            p = pq[:, c * 128:(c + 1) * 128]
            p4 = p.reshape(16, 5, 8, 128)
            t4 = (p * zb_v[...]).reshape(16, 5, 8, 128)
            sa = t4[:, 0] + t4[:, 1] + jnp.where(low, t4[:, 2], 0.0)
            sb = t4[:, 3] + t4[:, 4] + jnp.where(low, 0.0, t4[:, 2])
            ra = _recip(jnp.broadcast_to(jnp.sum(sa, axis=1, keepdims=True) + 1e-6, sa.shape))
            rb = _recip(jnp.broadcast_to(jnp.sum(sb, axis=1, keepdims=True) + 1e-6, sb.shape))
            o4 = jnp.stack([p4[:, 0] * ra, p4[:, 1] * ra, p4[:, 2] * jnp.where(low, ra, rb),
                            p4[:, 3] * rb, p4[:, 4] * rb], axis=1)
            cols.append(o4.reshape(D, 128))
        oT = jnp.concatenate(cols, axis=1).astype(BF)
        at = lax.dot_general(oT, m_v[...], TN, preferred_element_type=F32)
        for c in range(T // LC):
            r = pl.ds(t * T + c * LC, LC)
            hc = x_v[r, :].astype(F32) + at[c * LC:(c + 1) * LC]
            h_v[r, :] = hc
            if t == 0:
                hn_v[r, :] = _ln(hc).astype(BF)

    pqs = {t: qproj(t) for t in range(AHEAD)}
    gb = st["g"].astype(BF)
    parts = []
    for j, (lo, hi) in enumerate(RNG):
        kv = _dot(gb[lo:hi, :], wv_v[:, j * 128:(j + 1) * 128])
        ri = lax.broadcasted_iota(jnp.int32, kv.shape, 0) + lo
        ci = lax.broadcasted_iota(jnp.int32, kv.shape, 1) + j * 128
        kvb = jnp.where(_head(ri) == _head(ci), kv, 0.0).astype(BF)
        parts.append(_dot(kvb, wo_v[j * 128:(j + 1) * 128, :]))
    m_v[0:112, :] = parts[0][0:112].astype(BF)
    for j in range(1, 5):
        lo, hi = RNG[j]
        off = lo - RNG[j - 1][0]
        m_v[lo:lo + 32, :] = (parts[j - 1][off:off + 32] + parts[j][0:32]).astype(BF)
        end = hi - 32 if j < 4 else hi
        m_v[lo + 32:end, :] = parts[j][32:end - lo].astype(BF)
    zb_v[...] = jnp.broadcast_to(jnp.sum(st["z"], axis=1, keepdims=True), (D, 128))

    for t in range(N):
        if t + AHEAD < N:
            pqs[t + AHEAD] = qproj(t + AHEAD)
        attn(t, pqs.pop(t))

    for c in (cwg, cwu, cwd):
        c.wait()

    def ffn(t, carry):
        r = pl.ds(pl.multiple_of(t * T, T), T)
        hn = hn_v[...]
        gate = _dot(hn, wg_v[...])
        up = _dot(hn, wu_v[...])
        a = jnp.where(gate > 0, gate * up, 0.0).astype(BF)
        tn = jnp.minimum(t + 1, N - 1)
        for c in range(T // LC):
            rn = pl.ds(pl.multiple_of(tn * T + c * LC, LC), LC)
            hn_v[c * LC:(c + 1) * LC, :] = _ln(h_v[rn, :]).astype(BF)
        o_v[r, :] = (h_v[r, :] + _dot(a, wd_v[...])).astype(BF)
        cp(o_v.at[r], out_hbm.at[r], osems.at[t]).start()
        return carry

    lax.fori_loop(0, N, ffn, 0)
    for t in range(N):
        r = pl.ds(t * T, T)
        cp(o_v.at[r], out_hbm.at[r], osems.at[t]).wait()


@jax.jit
def pallas_sequential_preLN__linear_attn_block__glu_gated_reglu__prompt_kernel(
    A_x: jax.Array,
    A_wqkv: jax.Array,
    A_wo: jax.Array,
    B_x: jax.Array,
    B_W_gate: jax.Array,
    B_W_up: jax.Array,
    B_W_down: jax.Array,
):
    del B_x
    assert A_x.shape == (1, S, D) and B_W_gate.shape == (D, F)
    any_spec = pl.BlockSpec(memory_space=pl.ANY)
    out = pl.pallas_call(
        _kernel,
        grid=(1,),
        out_shape=jax.ShapeDtypeStruct((S, D), BF),
        in_specs=[any_spec] * 6,
        out_specs=any_spec,
        scratch_shapes=[
            pltpu.VMEM((S, D), BF),
            pltpu.VMEM((D, D), BF), pltpu.VMEM((D, D), BF),
            pltpu.VMEM((D, D), BF), pltpu.VMEM((D, D), BF),
            pltpu.VMEM((D, F), BF), pltpu.VMEM((D, F), BF),
            pltpu.VMEM((F, D), BF),
            pltpu.VMEM((D, D), BF), pltpu.VMEM((D, D), BF),
            pltpu.VMEM((S, D), BF),
            pltpu.VMEM((D, D), BF), pltpu.VMEM((D, 128), F32),
            pltpu.VMEM((S, D), F32), pltpu.VMEM((T, D), BF),
            pltpu.VMEM((S, D), BF),
            pltpu.SemaphoreType.DMA((10,)),
            pltpu.SemaphoreType.DMA((N,)),
        ],
        compiler_params=pltpu.CompilerParams(vmem_limit_bytes=100 * 1024 * 1024),
    )(A_x.reshape(S, D), A_wqkv, A_wo, B_W_gate, B_W_up, B_W_down)
    return out.reshape(1, S, D)
```
